```python
import os as _os
_os.environ.setdefault("JAX_PLATFORMS", "cpu")
import jax
import jax.numpy as jnp

def _softmax(x, axis=-1):
    return jax.nn.softmax(x, axis=axis)
def _gelu(x):
    return jax.nn.gelu(x, approximate=True)
def _silu(x):
    return jax.nn.silu(x)
def _sigmoid(x):
    return jax.nn.sigmoid(x)
def _layernorm(x, axis=-1, eps=1e-5):
    m = jnp.mean(x, axis=axis, keepdims=True)
    v = jnp.var(x, axis=axis, keepdims=True)
    return (x - m) / jnp.sqrt(v + eps)
def _scatter_add(tgt, idx, src, axis=0):
    return tgt.at[idx].add(src)
def _segment_sum(src, seg, n):
    return jax.ops.segment_sum(src, seg, n)
class _Rng:
    def __init__(self, key):
        self._k = key
    def _next(self):
        self._k, sub = jax.random.split(self._k)
        return sub
    def normal(self, shape):
        return jax.random.normal(self._next(), shape, dtype=jnp.bfloat16)
    def randint(self, lo, hi, shape):
        return jax.random.randint(self._next(), shape, lo, hi, dtype=jnp.int32)
    def uniform(self, shape, lo=0.0, hi=1.0):
        return jax.random.uniform(self._next(), shape, jnp.bfloat16, lo, hi)
    def permutation(self, n):
        return jax.random.permutation(self._next(), n)


kernel_name = 'gated_mix__sliding_block_cached__dense_activation_silu__decode'

def setup_inputs():
    _rng = _Rng(jax.random.key(int.from_bytes(__import__("os").urandom(4), "little")))
    _w = (lambda a: (lambda t: t.astype(jnp.bfloat16) if jnp.issubdtype(t.dtype, jnp.floating) else t)(jnp.asarray(a)))
    def _A_setup():
        B, Sq, D = 2, 1, 1024
        Hq, Hkv, Sk, Dh = 32, 4, 32768, 128
        assert Hq % Hkv == 0, (Hq, Hkv)
        return {
            "x": _w((lambda *s: _rng.normal(s) * 0.05)(B, Sq, D)),
            "k_cache": _w((lambda *s: _rng.normal(s) * 3.2)(B, Hkv, Sk, Dh)),
            "v_cache": _w((lambda *s: _rng.normal(s) * 0.05)(B, Hkv, Sk, Dh)),
            "wq": _w((lambda *s: _rng.normal(s) * 3.2)(D, Hq * Dh) * (D ** -0.5)),
            "wo": _w((lambda *s: _rng.normal(s) * 0.05)(Hq * Dh, D) * ((Hq * Dh) ** -0.5)),
        }
    _A_in = _A_setup()

    def _B_setup():
        B, S, D, F = 2, 1, 1024, 3584
        return {
            "x": _w((lambda *s: _rng.normal(s) * 0.05)(B, S, D)),
            "w1": _w((lambda *s: _rng.normal(s) * 0.05)(D, F) * (D ** -0.5)),
            "w2": _w((lambda *s: _rng.normal(s) * 0.05)(F, D) * (F ** -0.5)),
        }
    _B_in = _B_setup()

    return {
        "A_x": _A_in["x"],
        "A_k_cache": _A_in["k_cache"],
        "A_v_cache": _A_in["v_cache"],
        "A_wq": _A_in["wq"],
        "A_wo": _A_in["wo"],
        "B_x": _B_in["x"],
        "B_w1": _B_in["w1"],
        "B_w2": _B_in["w2"],
        "gate_w": _w((lambda *s: _rng.normal(s) * 0.05)(1024) * 16.0),
    }

def reference(A_x, A_k_cache, A_v_cache, A_wq, A_wo, B_x, B_w1, B_w2, gate_w):
    def _A_ref(x, k_cache, v_cache, wq, wo):
        B, Sq, D = x.shape
        Hq, Dh = 32, 128
        Hkv, Sk = k_cache.shape[1], k_cache.shape[2]
        W = min(4096, max(256, Sk // 4))
        rep = Hq // Hkv
        q = (lambda x, *d: x.transpose(*d))((x @ wq).reshape(B, Sq, Hq, Dh), 0, 2, 1, 3)
        k = jnp.repeat(k_cache[:, :, Sk - W:, :], rep, axis=1)
        v = jnp.repeat(v_cache[:, :, Sk - W:, :], rep, axis=1)
        scores = jnp.einsum("bhqd,bhkd->bhqk", q, k) * (Dh ** -0.5)
        p = _softmax(scores, axis=-1)
        o = jnp.einsum("bhqk,bhkd->bhqd", p, v)
        return (lambda x, *d: x.transpose(*d))(o, 0, 2, 1, 3).reshape(B, Sq, Hq * Dh) @ wo

    def _B_ref(x, w1, w2):
        h = jnp.einsum("bsd,df->bsf", x, w1)
        h = _silu(h)
        out = jnp.einsum("bsf,fd->bsd", h, w2)
        return out

    x = A_x
    g = _sigmoid((x * gate_w).sum(-1, keepdims=True))
    a = _A_ref(x, A_k_cache, A_v_cache, A_wq, A_wo)
    b = _B_ref(x, B_w1, B_w2)
    return g * a + (1 - g) * b
```

```python
import jax
import jax.numpy as jnp
import jax.experimental.pallas as pl
import jax.experimental.pallas.tpu as pltpu

_HQ = 32
_BF = jnp.bfloat16
_F32 = jnp.float32


def _build(rows_q=32, rows_kv=1024, rows_o=128, rows_1=32, rows_2=128, window=8, pri=True):
    def fn(x, k_cache, v_cache, wq, wo, b_x, w1, w2, gate_w):
        del b_x
        B, _, D = x.shape
        _, Hkv, Sk, Dh = k_cache.shape
        F = w1.shape[1]
        rep = _HQ // Hkv
        W = min(4096, max(256, Sk // 4))
        R = B * rep
        scale = Dh ** -0.5

        def kernel(x_h, k_h, v_h, wq_h, wo_h, w1_h, w2_h, g_h, o_ref,
                   x_v, g_v, k_v, v_v, wq_v, wo_v, w1_v, w2_v, sems, ssem):
            pairs = []
            for i in range(0, D, rows_q):
                pairs.append((wq_h.at[pl.ds(i, rows_q)], wq_v.at[pl.ds(i, rows_q)]))
            for c_h, c_v in ((k_h, k_v), (v_h, v_v)):
                for h in range(Hkv):
                    for b in range(B):
                        for i in range(0, W, rows_kv):
                            pairs.append((c_h.at[b, h, pl.ds(Sk - W + i, rows_kv)],
                                          c_v.at[b, h, pl.ds(i, rows_kv)]))
            for s, d, n, r in ((wo_h, wo_v, _HQ * Dh, rows_o), (w1_h, w1_v, D, rows_1),
                               (w2_h, w2_v, F, rows_2)):
                for i in range(0, n, r):
                    pairs.append((s.at[pl.ds(i, r)], d.at[pl.ds(i, r)]))
            copies = [pltpu.make_async_copy(s, d, sems.at[i % window])
                      for i, (s, d) in enumerate(pairs)]

            def start(i):
                copies[i].start(priority=i % 2 if pri else 0)

            cx = pltpu.make_async_copy(x_h, x_v, ssem.at[0])
            cg = pltpu.make_async_copy(g_h, g_v, ssem.at[1])
            start(0)
            cx.start()
            cg.start()
            for i in range(1, window):
                start(i)
            pos = [0]

            def advance():
                i = pos[0]
                copies[i].wait()
                if i + window < len(copies):
                    start(i + window)
                pos[0] = i + 1

            cx.wait()
            cg.wait()
            xf = jnp.concatenate(
                [jnp.broadcast_to(x_v[...].astype(_F32)[b:b + 1], (rep, D)) for b in range(B)], axis=0)
            gw = g_v[...].astype(_F32).reshape(1, D)
            g = jax.nn.sigmoid(jnp.sum(xf * gw, axis=-1, keepdims=True))
            xb = xf.astype(_BF)
            step = 128

            q = jnp.zeros((R, _HQ * Dh), _F32)
            for i in range(0, D, max(rows_q, step)):
                n = max(rows_q, step)
                for _ in range(n // rows_q):
                    advance()
                q += jnp.dot(xb[:, i:i + n], wq_v[i:i + n, :], preferred_element_type=_F32)

            row = jax.lax.broadcasted_iota(jnp.int32, (R, Dh), 0) % rep
            ps, ls = [], []
            for h in range(Hkv):
                qh = q[:, h * rep * Dh:(h * rep + 1) * Dh]
                for r in range(1, rep):
                    qh = jnp.where(row == r, q[:, (h * rep + r) * Dh:(h * rep + r + 1) * Dh], qh)
                for b in range(B):
                    for _ in range(W // rows_kv):
                        advance()
                    qb = qh[b * rep:(b + 1) * rep].astype(_BF)
                    s = jax.lax.dot_general(qb, k_v[b, h], (((1,), (1,)), ((), ())),
                                            preferred_element_type=_F32) * scale
                    p = jnp.exp(s - jnp.max(s, axis=-1, keepdims=True))
                    ls.append(jnp.sum(p, axis=-1, keepdims=True))
                    ps.append(p.astype(_BF))

            lhs = []
            for h in range(Hkv):
                os_ = []
                for b in range(B):
                    for _ in range(W // rows_kv):
                        advance()
                    j = h * B + b
                    os_.append(jnp.dot(ps[j], v_v[b, h], preferred_element_type=_F32) / ls[j])
                oh = jnp.concatenate(os_, axis=0)
                for r in range(rep):
                    lhs.append(jnp.where(row == r, oh, 0.0).astype(_BF))
            lhs = jnp.concatenate(lhs, axis=1)

            a = jnp.zeros((R, D), _F32)
            for i in range(0, _HQ * Dh, max(rows_o, step)):
                n = max(rows_o, step)
                for _ in range(n // rows_o):
                    advance()
                a += jnp.dot(lhs[:, i:i + n], wo_v[i:i + n, :], preferred_element_type=_F32)

            hid = jnp.zeros((R, F), _F32)
            for i in range(0, D, max(rows_1, step)):
                n = max(rows_1, step)
                for _ in range(n // rows_1):
                    advance()
                hid += jnp.dot(xb[:, i:i + n], w1_v[i:i + n, :], preferred_element_type=_F32)
            hid = (hid * jax.nn.sigmoid(hid)).astype(_BF)

            y = jnp.zeros((R, D), _F32)
            for i in range(0, F, max(rows_2, step)):
                n = max(rows_2, step)
                for _ in range(n // rows_2):
                    advance()
                y += jnp.dot(hid[:, i:i + n], w2_v[i:i + n, :], preferred_element_type=_F32)

            for b in range(B):
                ab = jnp.sum(a[b * rep:(b + 1) * rep], axis=0, keepdims=True)
                gb = g[b * rep:b * rep + 1]
                o_ref[b:b + 1, :] = (gb * ab + (1.0 - gb) * y[b * rep:b * rep + 1]).astype(o_ref.dtype)

        return pl.pallas_call(
            kernel,
            out_shape=jax.ShapeDtypeStruct((B, D), x.dtype),
            in_specs=[pl.BlockSpec(memory_space=pltpu.HBM)] * 8,
            out_specs=pl.BlockSpec(memory_space=pltpu.VMEM),
            scratch_shapes=[
                pltpu.VMEM((B, D), x.dtype),
                pltpu.VMEM(gate_w.shape, gate_w.dtype),
                pltpu.VMEM((B, Hkv, W, Dh), k_cache.dtype),
                pltpu.VMEM((B, Hkv, W, Dh), v_cache.dtype),
                pltpu.VMEM(wq.shape, wq.dtype),
                pltpu.VMEM(wo.shape, wo.dtype),
                pltpu.VMEM(w1.shape, w1.dtype),
                pltpu.VMEM(w2.shape, w2.dtype),
                pltpu.SemaphoreType.DMA((window,)),
                pltpu.SemaphoreType.DMA((2,)),
            ],
            compiler_params=pltpu.CompilerParams(vmem_limit_bytes=100 * 2**20),
        )(x.reshape(B, D), k_cache, v_cache, wq, wo, w1, w2, gate_w).reshape(x.shape)

    return fn


@jax.jit
def pallas_gated_mix__sliding_block_cached__dense_activation_silu__decode_kernel(
    A_x: jax.Array,
    A_k_cache: jax.Array,
    A_v_cache: jax.Array,
    A_wq: jax.Array,
    A_wo: jax.Array,
    B_x: jax.Array,
    B_w1: jax.Array,
    B_w2: jax.Array,
    gate_w: jax.Array,
):
    return _build()(A_x, A_k_cache, A_v_cache, A_wq, A_wo, B_x, B_w1, B_w2, gate_w)
```
